```python
import os as _os
_os.environ.setdefault("JAX_PLATFORMS", "cpu")
import jax
import jax.numpy as jnp

def _softmax(x, axis=-1):
    return jax.nn.softmax(x, axis=axis)
def _gelu(x):
    return jax.nn.gelu(x, approximate=True)
def _silu(x):
    return jax.nn.silu(x)
def _sigmoid(x):
    return jax.nn.sigmoid(x)
def _layernorm(x, axis=-1, eps=1e-5):
    m = jnp.mean(x, axis=axis, keepdims=True)
    v = jnp.var(x, axis=axis, keepdims=True)
    return (x - m) / jnp.sqrt(v + eps)
def _scatter_add(tgt, idx, src, axis=0):
    return tgt.at[idx].add(src)
def _segment_sum(src, seg, n):
    return jax.ops.segment_sum(src, seg, n)
class _Rng:
    def __init__(self, key):
        self._k = key
    def _next(self):
        self._k, sub = jax.random.split(self._k)
        return sub
    def normal(self, shape):
        return jax.random.normal(self._next(), shape, dtype=jnp.bfloat16)
    def randint(self, lo, hi, shape):
        return jax.random.randint(self._next(), shape, lo, hi, dtype=jnp.int32)
    def uniform(self, shape, lo=0.0, hi=1.0):
        return jax.random.uniform(self._next(), shape, jnp.bfloat16, lo, hi)
    def permutation(self, n):
        return jax.random.permutation(self._next(), n)


kernel_name = 'concat_heads__sliding_block_cached__compressed_kv_cla__decode'

def setup_inputs():
    _rng = _Rng(jax.random.key(int.from_bytes(__import__("os").urandom(4), "little")))
    _w = (lambda a: (lambda t: t.astype(jnp.bfloat16) if jnp.issubdtype(t.dtype, jnp.floating) else t)(jnp.asarray(a)))
    def _A_setup():
        B, Sq, D = 1, 1, 512
        Hq, Hkv, Sk, Dh = 32, 32, 4096, 128
        assert Hq % Hkv == 0, (Hq, Hkv)
        return {
            "x": _w((lambda *s: _rng.normal(s) * 0.8)(B, Sq, D)),
            "k_cache": _w((lambda *s: _rng.normal(s) * 0.8)(B, Hkv, Sk, Dh)),
            "v_cache": _w((lambda *s: _rng.normal(s) * 0.05)(B, Hkv, Sk, Dh)),
            "wq": _w((lambda *s: _rng.normal(s) * 0.8)(D, Hq * Dh) * (D ** -0.5)),
            "wo": _w((lambda *s: _rng.normal(s) * 0.05)(Hq * Dh, D) * ((Hq * Dh) ** -0.5)),
        }
    _A_in = _A_setup()

    def _B_setup():
        B, H, Sq, Sk, D, M = 1, 32, 1, 4096, 128, 512
        Dc = 4 * D
        return {
            "x": _w((lambda *s: _rng.normal(s) * 1.6)(B, Sq, M)),
            "c_kv": _w((lambda *s: _rng.normal(s) * 0.1)(B, Sk, Dc)),
            "w_q": _w((lambda *s: _rng.normal(s) * 1.6)(M, H, D) * (M ** -0.5)),
            "w_uk": _w((lambda *s: _rng.normal(s) * 1.6)(Dc, H, D) * (Dc ** -0.5)),
            "w_uv": _w((lambda *s: _rng.normal(s) * 0.1)(Dc, H, D) * (Dc ** -0.5)),
            "w_o": _w((lambda *s: _rng.normal(s) * 0.1)(H, D, M) * ((H * D) ** -0.5)),
        }
    _B_in = _B_setup()

    return {
        "A_x": _A_in["x"],
        "A_k_cache": _A_in["k_cache"],
        "A_v_cache": _A_in["v_cache"],
        "A_wq": _A_in["wq"],
        "A_wo": _A_in["wo"],
        "B_x": _B_in["x"],
        "B_c_kv": _B_in["c_kv"],
        "B_w_q": _B_in["w_q"],
        "B_w_uk": _B_in["w_uk"],
        "B_w_uv": _B_in["w_uv"],
        "B_w_o": _B_in["w_o"],
    }

def reference(A_x, A_k_cache, A_v_cache, A_wq, A_wo, B_x, B_c_kv, B_w_q, B_w_uk, B_w_uv, B_w_o):
    def _A_ref(x, k_cache, v_cache, wq, wo):
        B, Sq, D = x.shape
        Hq, Dh = 32, 128
        Hkv, Sk = k_cache.shape[1], k_cache.shape[2]
        W = min(4096, max(256, Sk // 4))
        rep = Hq // Hkv
        q = (lambda x, *d: x.transpose(*d))((x @ wq).reshape(B, Sq, Hq, Dh), 0, 2, 1, 3)
        k = jnp.repeat(k_cache[:, :, Sk - W:, :], rep, axis=1)
        v = jnp.repeat(v_cache[:, :, Sk - W:, :], rep, axis=1)
        scores = jnp.einsum("bhqd,bhkd->bhqk", q, k) * (Dh ** -0.5)
        p = _softmax(scores, axis=-1)
        o = jnp.einsum("bhqk,bhkd->bhqd", p, v)
        return (lambda x, *d: x.transpose(*d))(o, 0, 2, 1, 3).reshape(B, Sq, Hq * Dh) @ wo

    def _B_ref(x, c_kv, w_q, w_uk, w_uv, w_o):
        B, Sq, M = x.shape[0], x.shape[1], x.shape[2]
        Sk = c_kv.shape[1]
        H, D = w_q.shape[1], w_q.shape[2]
        q = jnp.einsum("bqm,mhd->bhqd", x, w_q)
        k = jnp.einsum("bkc,chd->bhkd", c_kv, w_uk)
        v = jnp.einsum("bkc,chd->bhkd", c_kv, w_uv)
        scores = jnp.einsum("bhqd,bhkd->bhqk", q, k) * (D ** -0.5)
        off = Sk - Sq
        qi = jnp.arange(Sq)[:, None]
        kj = jnp.arange(Sk)[None, :]
        cmask = kj <= (qi + off)
        scores = jnp.where(cmask[None, None], scores, -1e9)
        p = _softmax(scores, axis=-1)
        ctx = jnp.einsum("bhqk,bhkd->bhqd", p, v)
        return jnp.einsum("bhqd,hdm->bqm", ctx, w_o)

    a = _A_ref(A_x, A_k_cache, A_v_cache, A_wq, A_wo)
    b = _B_ref(B_x, B_c_kv, B_w_q, B_w_uk, B_w_uv, B_w_o)
    return jnp.concatenate([a, b], axis=-1)
```

```python
import functools
import jax
import jax.numpy as jnp
from jax import lax
from jax.experimental import pallas as pl
from jax.experimental.pallas import tpu as pltpu

_BF = jnp.bfloat16
_F32 = jnp.float32
_NT = (((1,), (1,)), ((), ()))


def _dot(a, b):
    return jnp.dot(a, b, preferred_element_type=_F32)


def _dot_nt(a, b):
    return lax.dot_general(a, b, _NT, preferred_element_type=_F32)


def _build(DEPTH=8):
    H, D, M, C, SK, W = 32, 128, 512, 512, 4096, 1024
    NCH = 16
    scale = D ** -0.5

    def kernel(ax, kc, vc, wq, wo, bx, ckv, bwq, wuk, wuv, bwo, out,
               axb, bxb, kb, vb, wqb, wob, cb, bwqb, wukb, wuvb, bwob,
               g_ref, qa_ref, sb_ref, accb_ref, qA_ref, sA_ref, oA_ref, ctx_ref, sems, xsems):
        w0 = kc.shape[2] - W

        def slab(src, dst):
            return lambda i: (src.at[:, pl.ds(i * 8, 8)], dst.at[:, pl.ds(i * 8, 8)])

        def rows(src, dst):
            return lambda i: (src.at[pl.ds(pl.multiple_of(i * 256, 256), 256), :], dst.at[i])

        def head(src, dst):
            return lambda i: (src.at[0, i, pl.ds(w0, W), :], dst.at[i])

        phases = [
            (slab(bwq, bwqb), NCH),
            (slab(wuk, wukb), NCH),
            (rows(ckv, cb), NCH),
            (lambda i: (wq.at[:, pl.ds(pl.multiple_of(i * 256, 256), 256)], wqb.at[i]), NCH),
            (slab(wuv, wuvb), NCH),
            (head(kc, kb), H),
            (rows(bwo, bwob), NCH),
            (head(vc, vb), H),
            (rows(wo, wob), NCH),
        ]
        offs = [0]
        for _, n in phases:
            offs.append(offs[-1] + n)

        def copy(p, i):
            src, dst = phases[p][0](i)
            return pltpu.make_async_copy(src, dst, sems.at[(offs[p] + i) % DEPTH])

        def advance(p, i, parity):
            copy(p, i).wait()
            n = phases[p][1]
            prio = (parity + DEPTH) % 2

            @pl.when(i + DEPTH < n)
            def _():
                copy(p, i + DEPTH).start(priority=prio)

            if p + 1 < len(phases):
                @pl.when(i + DEPTH >= n)
                def _():
                    copy(p + 1, i + DEPTH - n).start(priority=prio)

        def run_phase(p, step, carry):
            def body(j, c):
                for par in range(2):
                    i = 2 * j + par
                    advance(p, i, par)
                    c = step(i, c)
                return c
            return lax.fori_loop(0, phases[p][1] // 2, body, carry)

        xcopies = [pltpu.make_async_copy(bx, bxb, xsems.at[0]), pltpu.make_async_copy(ax, axb, xsems.at[1])]
        copy(0, 0).start(priority=0)
        copy(0, 1).start(priority=1)
        xcopies[0].start()
        xcopies[1].start()
        for i in range(2, DEPTH):
            copy(0, i).start(priority=i % 2)

        row = lax.broadcasted_iota(jnp.int32, (H, 128), 0)
        lane = lax.broadcasted_iota(jnp.int32, (H, 128), 1)
        diag = (lane % H) == row

        def stage_coeffs(v):
            g_ref[...] = jnp.concatenate([v[:, 128 * i:128 * (i + 1)] for i in range(4)], axis=0).T

        def slab_weights(buf, i):
            return jnp.concatenate([buf[q, i * 8 + j] for j in range(8) for q in range(4)], axis=0)

        def contract_major(buf):
            def step(i, acc):
                gg = g_ref[pl.ds(pl.multiple_of(i * 8, 8), 8), :]
                s = jnp.concatenate(
                    [jnp.where(diag, jnp.broadcast_to(gg[j:j + 1, :], (H, 128)), 0.0).astype(_BF) for j in range(8)], axis=1)
                return acc + _dot(s, slab_weights(buf, i))
            return step

        xcopies[0].wait()
        stage_coeffs(jnp.broadcast_to(bxb[...].astype(_F32), (H, M)))
        qB = run_phase(0, contract_major(bwqb), jnp.zeros((H, D), _F32)).astype(_BF)

        def uk_step(i, c):
            r = _dot_nt(qB, slab_weights(wukb, i))
            rows_ = [jnp.sum(jnp.where(diag, r[:, 128 * j:128 * (j + 1)], 0.0), axis=0, keepdims=True) for j in range(8)]
            g_ref[pl.ds(pl.multiple_of(i * 8, 8), 8), :] = jnp.concatenate(rows_, axis=0)
            return c
        run_phase(1, uk_step, 0)
        gt = g_ref[...].T
        qa_ref[...] = jnp.concatenate([gt[H * i:H * (i + 1), :] for i in range(4)], axis=1).astype(_BF)

        def sc_step(i, m):
            s = _dot_nt(qa_ref[...], cb[i]) * scale
            sb_ref[i] = s
            return jnp.maximum(m, jnp.maximum(s[:, :128], s[:, 128:]))
        mB = run_phase(2, sc_step, jnp.full((H, 128), -jnp.inf, _F32))
        mB = jnp.broadcast_to(jnp.max(mB, axis=1, keepdims=True), (H, 128))

        xcopies[1].wait()
        accb_ref[...] = jnp.zeros_like(accb_ref)

        def wq_step(i, l):
            q = _dot(axb[...], wqb[i])
            qA_ref[pl.ds(2 * i, 1), :] = q[:, :128]
            qA_ref[pl.ds(2 * i + 1, 1), :] = q[:, 128:]
            s = sb_ref[i]
            p0 = jnp.exp(s[:, :128] - mB)
            p1 = jnp.exp(s[:, 128:] - mB)
            accb_ref[...] += _dot(jnp.concatenate([p0, p1], axis=1).astype(_BF), cb[i])
            return l + (p0 + p1)
        lB = run_phase(3, wq_step, jnp.zeros((H, 128), _F32))
        lB = jnp.sum(lB, axis=1, keepdims=True)
        stage_coeffs(accb_ref[...] / lB)

        ctx_ref[...] = run_phase(4, contract_major(wuvb), jnp.zeros((H, D), _F32))

        def k_step(i, c):
            sA_ref[pl.ds(i, 1), :] = _dot_nt(qA_ref[pl.ds(i, 1), :].astype(_BF), kb[i]) * scale
            return c
        run_phase(5, k_step, 0)
        sA = sA_ref[...]
        pA = jnp.exp(sA - jnp.max(sA, axis=1, keepdims=True))
        sA_ref[...] = pA / jnp.sum(pA, axis=1, keepdims=True)

        def out_proj(src_ref, buf):
            def step(i, acc):
                o = jnp.concatenate([src_ref[pl.ds(2 * i, 1), :], src_ref[pl.ds(2 * i + 1, 1), :]], axis=1)
                return acc + _dot(o.astype(_BF), buf[i])
            return step

        oB = run_phase(6, out_proj(ctx_ref, bwob), jnp.zeros((1, M), _F32))
        out[:, M:] = oB.astype(_BF)

        def v_step(i, c):
            oA_ref[pl.ds(i, 1), :] = _dot(sA_ref[pl.ds(i, 1), :].astype(_BF), vb[i])
            return c
        run_phase(7, v_step, 0)

        oA = run_phase(8, out_proj(oA_ref, wob), jnp.zeros((1, M), _F32))
        out[:, :M] = oA.astype(_BF)

    hbm = pl.BlockSpec(memory_space=pltpu.HBM)
    V = pltpu.VMEM
    call = pl.pallas_call(
        kernel,
        in_specs=[hbm] * 11,
        out_specs=pl.BlockSpec(memory_space=pltpu.VMEM),
        out_shape=jax.ShapeDtypeStruct((1, 2 * M), _BF),
        scratch_shapes=[
            V((1, M), _BF), V((1, M), _BF),
            V((H, W, D), _BF), V((H, W, D), _BF),
            V((NCH, M, 256), _BF), V((NCH, 256, M), _BF), V((NCH, 256, C), _BF),
            V((4, 128, H, D), _BF), V((4, 128, H, D), _BF), V((4, 128, H, D), _BF),
            V((NCH, 256, M), _BF),
            V((128, 128), _F32), V((H, C), _BF), V((NCH, H, 256), _F32), V((H, C), _F32),
            V((H, D), _F32), V((H, W), _F32), V((H, D), _F32), V((H, D), _F32),
            pltpu.SemaphoreType.DMA((DEPTH,)), pltpu.SemaphoreType.DMA((2,)),
        ],
        compiler_params=pltpu.CompilerParams(vmem_limit_bytes=64 * 1024 * 1024),
    )

    def fn(A_x, A_k_cache, A_v_cache, A_wq, A_wo, B_x, B_c_kv, B_w_q, B_w_uk, B_w_uv, B_w_o):
        q4 = lambda w: w.reshape(4, 128, H, D)
        o = call(A_x.reshape(1, M), A_k_cache, A_v_cache, A_wq, A_wo, B_x.reshape(1, M), B_c_kv.reshape(SK, C),
                 q4(B_w_q), q4(B_w_uk), q4(B_w_uv), B_w_o.reshape(H * D, M))
        return o.reshape(1, 1, 2 * M)
    return fn


@jax.jit
def pallas_concat_heads__sliding_block_cached__compressed_kv_cla__decode_kernel(
    A_x, A_k_cache, A_v_cache, A_wq, A_wo, B_x, B_c_kv, B_w_q, B_w_uk, B_w_uv, B_w_o,
):
    return _build()(A_x, A_k_cache, A_v_cache, A_wq, A_wo, B_x, B_c_kv, B_w_q, B_w_uk, B_w_uv, B_w_o)
```

```python
import jax
import jax.numpy as jnp
from jax import lax
from jax.experimental import pallas as pl
from jax.experimental.pallas import tpu as pltpu

_BF = jnp.bfloat16
_F32 = jnp.float32

_H = 32
_D = 128
_M = 512
_C = 512
_SK = 4096
_W = 1024

_DEPTH = 11
_NSEM = 16
_NVPU = 5


def _dot(a, b):
    return jnp.dot(a, b, preferred_element_type=_F32)


def _dot_nt(a, b):
    return lax.dot_general(a, b, (((1,), (1,)), ((), ())), preferred_element_type=_F32)


def _ds(start, size):
    if not isinstance(start, int):
        start = pl.multiple_of(start, size)
    return pl.ds(start, size)


def _kernel(ax, kc, vc, wq, wo, bx, ckv, bwq, wuk, wuv, bwo, out,
            axb, bxb, kb, vb, wqb, wob, cb, bwqb, wukb, wuvb, bwob,
            g_ref, qa_ref, sb_ref, accb_ref, qA_ref, sA_ref, oA_ref, ctx_ref, yb_ref, sems, xsems):
    H, D, M, C = _H, _D, _M, _C
    w0 = _SK - _W
    scale = _D ** -0.5

    def slabs(src, dst):
        def lane(i):
            s = _ds(2 * i, 2)
            return [(src.at[u, s], dst.at[u, s]) for u in range(4)], dst.at[:, s]
        return lane

    def ckv_rows(i):
        j, e = i >> 2, i & 3
        return ([(ckv.at[u, _ds(16 * i, 16), :], cb.at[j, _ds(64 * e + 16 * u, 16), :]) for u in range(4)],
                cb.at[j, _ds(64 * e, 64), :])

    def bwo_rows(i):
        s = _ds(16 * i, 16)
        return [(bwo.at[u, s, :], bwob.at[u, s, :]) for u in range(4)], bwob.at[:, s, :]

    def wo_rows(i):
        return [(wo.at[u, _ds(16 * i, 16), :], wob.at[i, pl.ds(16 * u, 16), :]) for u in range(8)], wob.at[i]

    def wq_blocks(i):
        b, r = i >> 3, _ds(16 * (i & 7), 16)
        return [(wq.at[u, r, _ds(512 * b, 512)], wqb.at[b, u, r, :]) for u in range(4)], wqb.at[b, :, r, :]

    def heads(src, dst, first):
        def lane(i):
            i = i + first
            e, z, g, j = i & 1, (i >> 1) & 1, (i >> 2) & 3, i >> 4
            r = 128 * j + 64 * e
            return ([(src.at[0, 16 * z + 4 * u + g, _ds(w0 + r, 64), :], dst.at[g, 4 * z + u, _ds(r, 64), :])
                     for u in range(4)],
                    dst.at[g, _ds(4 * z, 4), _ds(r, 64), :])
        return lane

    stages = [
        ([wq_blocks, slabs(bwq, bwqb)], 64),
        ([heads(kc, kb, 0), slabs(wuk, wukb)], 64),
        ([heads(kc, kb, 64), ckv_rows], 64),
        ([heads(vc, vb, 0), slabs(wuv, wuvb)], 64),
        ([heads(vc, vb, 64), bwo_rows], 64),
        ([wo_rows], 32),
    ]

    def sem(i, lane_idx):
        return sems.at[(i & (_NSEM - 1)) + _NSEM * lane_idx]

    def start(p, i):
        per_lane = [[(s, d, sem(i, li)) for s, d in lane(i)[0]] for li, lane in enumerate(stages[p][0])]
        interleaved = [c for group in zip(*per_lane) for c in group]
        for n, (s, d, sm) in enumerate(interleaved):
            pltpu.make_async_copy(s, d, sm).start(priority=n % 2)

    def wait(p, i):
        for li, lane in enumerate(stages[p][0]):
            region = lane(i)[1]
            pltpu.make_async_copy(region, region, sem(i, li)).wait()

    def advance(p, i):
        wait(p, i)
        n, nxt = stages[p][1], i + _DEPTH

        @pl.when(nxt < n)
        def _():
            start(p, nxt)

        if p + 1 < len(stages):
            @pl.when(nxt >= n)
            def _():
                start(p + 1, nxt - n)

    def run(p, group, lo, hi, step, carry):
        def body(j, c):
            lax.fori_loop(0, group, lambda e, _: advance(p, group * j + e), None)
            return step(j, c)
        return lax.fori_loop(lo, hi, body, carry)

    x_copies = [pltpu.make_async_copy(bx, bxb, xsems.at[0]), pltpu.make_async_copy(ax, axb, xsems.at[1])]
    start(0, 0)
    for c in x_copies:
        c.start()
    lax.fori_loop(1, _DEPTH, lambda i, _: start(0, i), None)

    diag = (lax.broadcasted_iota(jnp.int32, (H, 128), 1) % H) == lax.broadcasted_iota(jnp.int32, (H, 128), 0)
    row8 = lax.broadcasted_iota(jnp.int32, (8, 128), 0)

    def slab_tiles(buf, j):
        return jnp.concatenate([buf[i, 8 * j + r] for r in range(8) for i in range(4)], axis=0)

    def stage_coeffs(v):
        g_ref[...] = jnp.concatenate([v[:, 128 * i:128 * (i + 1)] for i in range(4)], axis=0).T

    def contract_major(buf, j):
        g = g_ref[_ds(8 * j, 8), :]
        lhs = jnp.concatenate(
            [jnp.where(diag, jnp.broadcast_to(g[r:r + 1, :], (H, 128)), 0.0).astype(_BF) for r in range(8)], axis=1)
        return _dot(lhs, slab_tiles(buf, j))

    def k_step(n):
        g, j = n & 3, n >> 2
        r = _dot_nt(qA_ref[_ds(8 * g, 8), :].astype(_BF), kb[g, :, _ds(128 * j, 128), :].reshape(8 * 128, D))
        s = r[:, :128]
        for u in range(1, 8):
            s = jnp.where(row8 == u, r[:, 128 * u:128 * (u + 1)], s)
        sA_ref[j, _ds(8 * g, 8), :] = s * scale

    def v_step(n):
        g, j = n & 3, n >> 2
        p = sA_ref[j, _ds(8 * g, 8), :]
        lhs = jnp.concatenate([jnp.where(row8 == u, p, 0.0) for u in range(8)], axis=1).astype(_BF)
        oA_ref[_ds(8 * g, 8), :] += _dot(lhs, vb[g, :, _ds(128 * j, 128), :].reshape(8 * 128, D))

    for c in x_copies:
        c.wait()
    stage_coeffs(jnp.broadcast_to(bxb[...].astype(_F32), (H, M)))

    def step0(j, acc):
        q = _dot(axb[...], wqb[j].reshape(M, 512))
        for t in range(4):
            qA_ref[pl.ds(8 * t + j, 1), :] = q[:, 128 * t:128 * (t + 1)]
        return acc + (contract_major(bwqb, 2 * j) + contract_major(bwqb, 2 * j + 1))
    qB = run(0, 8, 0, 8, step0, jnp.zeros((H, D), _F32)).astype(_BF)

    def step1(j, c):
        k_step(j)
        r = _dot_nt(qB, slab_tiles(wukb, j))
        g_ref[_ds(8 * j, 8), :] = jnp.concatenate(
            [jnp.sum(jnp.where(diag, r[:, 128 * t:128 * (t + 1)], 0.0), axis=0, keepdims=True) for t in range(8)],
            axis=0)
        return c
    run(1, 4, 0, 16, step1, 0)
    gt = g_ref[...].T
    qa_ref[...] = jnp.concatenate([gt[H * i:H * (i + 1), :] for i in range(4)], axis=1).astype(_BF)

    def step2(j, m):
        k_step(j + 16)
        s = _dot_nt(qa_ref[...], cb[j]) * scale
        sb_ref[j] = s
        return jnp.maximum(m, jnp.maximum(s[:, :128], s[:, 128:]))
    mB = run(2, 4, 0, 16, step2, jnp.full((H, 128), -jnp.inf, _F32))
    mB = jnp.broadcast_to(jnp.max(mB, axis=1, keepdims=True), (H, 128))

    sA = sA_ref[...]
    pA = jnp.exp(sA - jnp.max(jnp.max(sA, axis=0), axis=1, keepdims=True)[None])
    sA_ref[...] = pA / jnp.sum(jnp.sum(pA, axis=0), axis=1, keepdims=True)[None]
    oA_ref[...] = jnp.zeros_like(oA_ref)
    accb_ref[...] = jnp.zeros_like(accb_ref)

    def step3a(j, l):
        v_step(j)
        ps = [jnp.exp(sb_ref[2 * j + (t >> 1), :, 128 * (t & 1):128 * (t & 1) + 128] - mB) for t in range(4)]
        accb_ref[...] += _dot(jnp.concatenate(ps, axis=1).astype(_BF), cb[pl.ds(2 * j, 2)].reshape(512, C))
        return l + ((ps[0] + ps[1]) + (ps[2] + ps[3]))
    lB = run(3, 4, 0, 8, step3a, jnp.zeros((H, 128), _F32))
    stage_coeffs(accb_ref[...] / jnp.sum(lB, axis=1, keepdims=True))

    def step3b(j, acc):
        v_step(j)
        return acc + (contract_major(wuvb, 2 * j - 16) + contract_major(wuvb, 2 * j - 15))
    ctx_ref[...] = run(3, 4, 8, 16, step3b, jnp.zeros((H, D), _F32))

    def step4(a, acc):
        v_step(2 * a + 16)
        v_step(2 * a + 17)
        ctx = jnp.concatenate([ctx_ref[pl.ds(8 * u + a, 1), :] for u in range(4)], axis=1)
        return acc + _dot(ctx.astype(_BF), bwob[:, _ds(128 * a, 128), :].reshape(512, M))
    out[:, M:] = run(4, 8, 0, 8, step4, jnp.zeros((1, M), _F32)).astype(_BF)

    shift = ((lax.broadcasted_iota(jnp.int32, (8, 128), 1) >> 4) - row8) & 7
    for a in range(4):
        o = oA_ref[pl.ds(8 * a, 8), :]
        l = o
        for d in range(1, 8):
            l = jnp.where(shift == d, pltpu.roll(pltpu.roll(o, 8 - d, 0), 16 * d, 1), l)
        oA_ref[pl.ds(8 * a, 8), :] = l
    n_mxu = 32 - _NVPU
    for e in range(_NVPU):
        yb_ref[e] = jnp.broadcast_to(oA_ref[pl.ds(n_mxu + e, 1), :], (128, 128)).T

    def wo_mxu(i0, n):
        o = jnp.concatenate([oA_ref[pl.ds(i0 + e, 1), :] for e in range(n)], axis=1)
        return _dot(o.astype(_BF), wob[pl.ds(i0, n)].reshape(128 * n, M))

    oA = run(5, 4, 0, n_mxu // 4, lambda j, acc: acc + wo_mxu(4 * j, 4), jnp.zeros((1, M), _F32))
    i0 = 4 * (n_mxu // 4)
    if i0 < n_mxu:
        for i in range(i0, n_mxu):
            wait(5, i)
        oA = oA + wo_mxu(i0, n_mxu - i0)
    for e in range(_NVPU):
        wait(5, n_mxu + e)
        acc = [None] * 4
        for r in range(16):
            y = yb_ref[e, pl.ds(8 * r, 8), :]
            for t in range(4):
                v = wob[n_mxu + e, pl.ds(8 * r, 8), pl.ds(128 * t, 128)].astype(_F32) * y
                acc[t] = v if acc[t] is None else acc[t] + v
        oA = oA + jnp.concatenate([jnp.sum(a, axis=0, keepdims=True) for a in acc], axis=1)
    out[:, :M] = oA.astype(_BF)


@jax.jit
def pallas_concat_heads__sliding_block_cached__compressed_kv_cla__decode_kernel(
    A_x: jax.Array,
    A_k_cache: jax.Array,
    A_v_cache: jax.Array,
    A_wq: jax.Array,
    A_wo: jax.Array,
    B_x: jax.Array,
    B_c_kv: jax.Array,
    B_w_q: jax.Array,
    B_w_uk: jax.Array,
    B_w_uv: jax.Array,
    B_w_o: jax.Array,
):
    H, D, M, C, W = _H, _D, _M, _C, _W
    assert A_k_cache.shape == A_v_cache.shape == (1, H, _SK, D) and B_c_kv.shape == (1, _SK, C)
    assert 4 * ((32 - _NVPU) // 4) + _DEPTH >= 32 and _DEPTH < _NSEM

    vmem = pltpu.VMEM
    out = pl.pallas_call(
        _kernel,
        in_specs=[pl.BlockSpec(memory_space=pltpu.HBM)] * 11,
        out_specs=pl.BlockSpec(memory_space=pltpu.VMEM),
        out_shape=jax.ShapeDtypeStruct((1, 2 * M), _BF),
        scratch_shapes=[
            vmem((1, M), _BF), vmem((1, M), _BF),
            vmem((4, 8, W, D), _BF), vmem((4, 8, W, D), _BF),
            vmem((8, 4, 128, 512), _BF), vmem((32, 128, M), _BF), vmem((16, 256, C), _BF),
            vmem((4, 128, H, D), _BF), vmem((4, 128, H, D), _BF), vmem((4, 128, H, D), _BF),
            vmem((4, 1024, M), _BF),
            vmem((128, 128), _F32), vmem((H, C), _BF), vmem((16, H, 256), _F32), vmem((H, C), _F32),
            vmem((H, D), _F32), vmem((8, H, 128), _F32), vmem((H, D), _F32), vmem((H, D), _F32),
            vmem((_NVPU, 128, 128), _F32),
            pltpu.SemaphoreType.DMA((2 * _NSEM,)), pltpu.SemaphoreType.DMA((2,)),
        ],
        compiler_params=pltpu.CompilerParams(
            vmem_limit_bytes=64 * 1024 * 1024,
            disable_bounds_checks=True,
            disable_semaphore_checks=True,
        ),
    )(
        A_x.reshape(1, M), A_k_cache, A_v_cache, A_wq.reshape(4, 128, H * D), A_wo.reshape(8, 512, M),
        B_x.reshape(1, M), B_c_kv.reshape(4, 1024, C),
        B_w_q.reshape(4, 128, H, D), B_w_uk.reshape(4, 128, H, D), B_w_uv.reshape(4, 128, H, D),
        B_w_o.reshape(4, 1024, M),
    )
    return out.reshape(1, 1, 2 * M)
```

```python
import jax
import jax.numpy as jnp
from jax import lax
from jax.experimental import pallas as pl
from jax.experimental.pallas import tpu as pltpu

_BF = jnp.bfloat16
_F32 = jnp.float32

_H = 32
_D = 128
_M = 512
_C = 512
_SK = 4096
_W = 1024

_DEPTH = 12
_QUEUE = (1, 1, 0, 1, 1, 1, 0, 1)
_NSEM = 16
_NVPU = 6


def _dot(a, b):
    return jnp.dot(a, b, preferred_element_type=_F32)


def _dot_nt(a, b):
    return lax.dot_general(a, b, (((1,), (1,)), ((), ())), preferred_element_type=_F32)


def _ds(start, size):
    if not isinstance(start, int):
        start = pl.multiple_of(start, size)
    return pl.ds(start, size)


def _kernel(ax, kc, vc, wq, wo, bx, ckv, bwq, wuk, wuv, bwo, out,
            axb, bxb, kb, vb, wqb, wob, cb, bwqb, wukb, wuvb, bwob,
            g_ref, qa_ref, sb_ref, accb_ref, qA_ref, sA_ref, oA_ref, ctx_ref, xp_ref, yb_ref, sems, xsems):
    H, D, M, C = _H, _D, _M, _C
    w0 = _SK - _W
    scale = _D ** -0.5

    def slabs(src, dst):
        def lane(i):
            s = _ds(2 * i, 2)
            return [(src.at[u, s], dst.at[u, s]) for u in range(4)], dst.at[:, s]
        return lane

    def ckv_rows(i):
        j, e = i >> 2, i & 3
        return ([(ckv.at[u, _ds(16 * i, 16), :], cb.at[j, _ds(64 * e + 16 * u, 16), :]) for u in range(4)],
                cb.at[j, _ds(64 * e, 64), :])

    def bwo_rows(i):
        s = _ds(16 * i, 16)
        return [(bwo.at[u, s, :], bwob.at[u, s, :]) for u in range(4)], bwob.at[:, s, :]

    def wo_rows(i):
        return ([(wo.at[n, _ds(16 * i, 16), :], wob.at[i, pl.ds(16 * (4 * (n % 2) + n // 2), 16), :])
                 for n in range(8)], wob.at[i])

    def wq_rows(i):
        r, c = _ds(8 * (i >> 2), 8), _ds(1024 * (i & 3), 1024)
        return [(wq.at[u, r, c], wqb.at[u, r, c]) for u in range(4)], wqb.at[:, r, c]

    def heads(src, dst, first):
        def lane(i):
            i = i + first
            e, z, g, j = i & 1, (i >> 1) & 1, (i >> 2) & 3, i >> 4
            r = 128 * j + 64 * e
            return ([(src.at[0, 8 * u + 4 * z + g, _ds(w0 + r, 64), :], dst.at[g, 4 * z + u, _ds(r, 64), :])
                     for u in range(4)],
                    dst.at[g, _ds(4 * z, 4), _ds(r, 64), :])
        return lane

    stages = [
        ([slabs(bwq, bwqb), wq_rows], 64),
        ([slabs(wuk, wukb), heads(kc, kb, 0)], 64),
        ([ckv_rows, heads(kc, kb, 64)], 64),
        ([slabs(wuv, wuvb), heads(vc, vb, 0)], 64),
        ([bwo_rows, heads(vc, vb, 64)], 64),
        ([wo_rows], 32),
    ]

    def sem(i, lane_idx):
        return sems.at[(i & (_NSEM - 1)) + _NSEM * lane_idx]

    def start(p, i):
        per_lane = [[(s, d, sem(i, li)) for s, d in lane(i)[0]] for li, lane in enumerate(stages[p][0])]
        interleaved = [c for group in zip(*per_lane) for c in group]
        for n, (s, d, sm) in enumerate(interleaved):
            pltpu.make_async_copy(s, d, sm).start(priority=_QUEUE[n])

    def wait(p, i):
        for li, lane in enumerate(stages[p][0]):
            region = lane(i)[1]
            pltpu.make_async_copy(region, region, sem(i, li)).wait()

    def advance(p, i):
        wait(p, i)
        n, nxt = stages[p][1], i + _DEPTH

        @pl.when(nxt < n)
        def _():
            start(p, nxt)

        if p + 1 < len(stages):
            @pl.when(nxt >= n)
            def _():
                start(p + 1, nxt - n)

    def run(p, group, lo, hi, step, carry):
        def body(j, c):
            lax.fori_loop(0, group, lambda e, _: advance(p, group * j + e), None)
            return step(j, c)
        return lax.fori_loop(lo, hi, body, carry)

    x_copies = [pltpu.make_async_copy(bx, bxb, xsems.at[0]), pltpu.make_async_copy(ax, axb, xsems.at[1])]
    start(0, 0)
    for c in x_copies:
        c.start()
    lax.fori_loop(1, _DEPTH, lambda i, _: start(0, i), None)

    diag = (lax.broadcasted_iota(jnp.int32, (H, 128), 1) % H) == lax.broadcasted_iota(jnp.int32, (H, 128), 0)
    row8 = lax.broadcasted_iota(jnp.int32, (8, 128), 0)

    shift = ((lax.broadcasted_iota(jnp.int32, (8, 128), 1) >> 4) - row8) & 7

    def block_transpose(o):
        l = o
        for d in range(1, 8):
            l = jnp.where(shift == d, pltpu.roll(pltpu.roll(o, 8 - d, 0), 16 * d, 1), l)
        return l

    def pick_rows(tiles):
        s = tiles[0]
        for v in range(1, len(tiles)):
            s = jnp.where(row8 == v, tiles[v], s)
        return s

    def slab_tiles(buf, j):
        return jnp.concatenate([buf[i, 8 * j + r] for r in range(8) for i in range(4)], axis=0)

    def stage_coeffs(v):
        g_ref[...] = jnp.concatenate([v[:, 128 * i:128 * (i + 1)] for i in range(4)], axis=0).T

    def contract_major(buf, j):
        g = g_ref[_ds(8 * j, 8), :]
        lhs = jnp.concatenate(
            [jnp.where(diag, jnp.broadcast_to(g[r:r + 1, :], (H, 128)), 0.0).astype(_BF) for r in range(8)], axis=1)
        return _dot(lhs, slab_tiles(buf, j))

    def k_step(n):
        g, j = n & 3, n >> 2
        r = _dot_nt(qA_ref[_ds(8 * g, 8), :].astype(_BF), kb[g, :, _ds(128 * j, 128), :].reshape(8 * 128, D))
        sA_ref[j, _ds(8 * g, 8), :] = pick_rows([r[:, 128 * v:128 * (v + 1)] for v in range(8)]) * scale

    def v_step(n):
        g, j = n & 3, n >> 2
        p = sA_ref[j, _ds(8 * g, 8), :]
        lhs = jnp.concatenate([jnp.where(row8 == v, p, 0.0) for v in range(8)], axis=1).astype(_BF)
        oA_ref[_ds(8 * g, 8), :] += _dot(lhs, vb[g, :, _ds(128 * j, 128), :].reshape(8 * 128, D))

    for c in x_copies:
        c.wait()
    stage_coeffs(jnp.broadcast_to(bxb[...].astype(_F32), (H, M)))

    xa = jnp.broadcast_to(axb[...].astype(_F32), (8, M))
    xp_ref[...] = block_transpose(pick_rows([xa[:, 128 * u:128 * (u + 1)] for u in range(4)]))

    def step0(j, carry):
        qA, qB = carry
        x = jnp.broadcast_to(xp_ref[pl.ds(j, 1), :], (8, 128))[:, :64]
        q = _dot(x.astype(_BF), wqb[:, _ds(16 * j, 16), :].reshape(64, H * D))
        q = jnp.concatenate(
            [pick_rows([q[:, D * h:D * (h + 1)] for h in [8 * (v % 4) + 4 * (v // 4) + g for v in range(8)]])
             for g in range(4)], axis=0)
        return qA + q, qB + (contract_major(bwqb, 2 * j) + contract_major(bwqb, 2 * j + 1))
    qA, qB = run(0, 8, 0, 8, step0, (jnp.zeros((H, D), _F32), jnp.zeros((H, D), _F32)))
    qA_ref[...] = qA
    qB = qB.astype(_BF)

    def step1(j, c):
        k_step(j)
        r = _dot_nt(qB, slab_tiles(wukb, j))
        g_ref[_ds(8 * j, 8), :] = jnp.concatenate(
            [jnp.sum(jnp.where(diag, r[:, 128 * t:128 * (t + 1)], 0.0), axis=0, keepdims=True) for t in range(8)],
            axis=0)
        return c
    run(1, 4, 0, 16, step1, 0)
    gt = g_ref[...].T
    qa_ref[...] = jnp.concatenate([gt[H * i:H * (i + 1), :] for i in range(4)], axis=1).astype(_BF)

    def step2(j, m):
        k_step(j + 16)
        s = _dot_nt(qa_ref[...], cb[j]) * scale
        sb_ref[j] = s
        return jnp.maximum(m, jnp.maximum(s[:, :128], s[:, 128:]))
    mB = run(2, 4, 0, 16, step2, jnp.full((H, 128), -jnp.inf, _F32))
    mB = jnp.broadcast_to(jnp.max(mB, axis=1, keepdims=True), (H, 128))

    sA = sA_ref[...]
    pA = jnp.exp(sA - jnp.max(jnp.max(sA, axis=0), axis=1, keepdims=True)[None])
    sA_ref[...] = pA / jnp.sum(jnp.sum(pA, axis=0), axis=1, keepdims=True)[None]
    oA_ref[...] = jnp.zeros_like(oA_ref)
    accb_ref[...] = jnp.zeros_like(accb_ref)

    def step3a(j, l):
        v_step(j)
        ps = [jnp.exp(sb_ref[2 * j + (t >> 1), :, 128 * (t & 1):128 * (t & 1) + 128] - mB) for t in range(4)]
        accb_ref[...] += _dot(jnp.concatenate(ps, axis=1).astype(_BF), cb[pl.ds(2 * j, 2)].reshape(512, C))
        return l + ((ps[0] + ps[1]) + (ps[2] + ps[3]))
    lB = run(3, 4, 0, 8, step3a, jnp.zeros((H, 128), _F32))
    stage_coeffs(accb_ref[...] / jnp.sum(lB, axis=1, keepdims=True))

    def step3b(j, acc):
        v_step(j)
        return acc + (contract_major(wuvb, 2 * j - 16) + contract_major(wuvb, 2 * j - 15))
    ctx_ref[...] = run(3, 4, 8, 16, step3b, jnp.zeros((H, D), _F32))

    def step4(a, acc):
        v_step(2 * a + 16)
        v_step(2 * a + 17)
        ctx = jnp.concatenate([ctx_ref[pl.ds(8 * u + a, 1), :] for u in range(4)], axis=1)
        return acc + _dot(ctx.astype(_BF), bwob[:, _ds(128 * a, 128), :].reshape(512, M))
    out[:, M:] = run(4, 8, 0, 8, step4, jnp.zeros((1, M), _F32)).astype(_BF)

    for g in range(4):
        oA_ref[pl.ds(8 * g, 8), :] = block_transpose(oA_ref[pl.ds(8 * g, 8), :])
    n_mxu = 32 - _NVPU
    for e in range(_NVPU):
        yb_ref[e] = jnp.broadcast_to(oA_ref[pl.ds(n_mxu + e, 1), :], (128, 128)).T

    def wo_mxu(i0, n):
        o = jnp.concatenate([oA_ref[pl.ds(i0 + e, 1), :] for e in range(n)], axis=1)
        return _dot(o.astype(_BF), wob[pl.ds(i0, n)].reshape(128 * n, M))

    oA = run(5, 4, 0, n_mxu // 4, lambda j, acc: acc + wo_mxu(4 * j, 4), jnp.zeros((1, M), _F32))
    i0 = 4 * (n_mxu // 4)
    if i0 < n_mxu:
        for i in range(i0, n_mxu):
            wait(5, i)
        oA = oA + wo_mxu(i0, n_mxu - i0)
    acc = [None] * 4
    for e in range(_NVPU):
        wait(5, n_mxu + e)
        for r in range(16):
            y = yb_ref[e, pl.ds(8 * r, 8), :]
            for t in range(4):
                v = wob[n_mxu + e, pl.ds(8 * r, 8), pl.ds(128 * t, 128)].astype(_F32) * y
                acc[t] = v if acc[t] is None else acc[t] + v
    oA = oA + jnp.concatenate([jnp.sum(a, axis=0, keepdims=True) for a in acc], axis=1)
    out[:, :M] = oA.astype(_BF)


@jax.jit
def pallas_concat_heads__sliding_block_cached__compressed_kv_cla__decode_kernel(
    A_x: jax.Array,
    A_k_cache: jax.Array,
    A_v_cache: jax.Array,
    A_wq: jax.Array,
    A_wo: jax.Array,
    B_x: jax.Array,
    B_c_kv: jax.Array,
    B_w_q: jax.Array,
    B_w_uk: jax.Array,
    B_w_uv: jax.Array,
    B_w_o: jax.Array,
):
    H, D, M, C, W = _H, _D, _M, _C, _W
    assert A_k_cache.shape == A_v_cache.shape == (1, H, _SK, D) and B_c_kv.shape == (1, _SK, C)
    assert 4 * ((32 - _NVPU) // 4) + _DEPTH >= 32 and _DEPTH < _NSEM

    vmem = pltpu.VMEM
    out = pl.pallas_call(
        _kernel,
        in_specs=[pl.BlockSpec(memory_space=pltpu.HBM)] * 11,
        out_specs=pl.BlockSpec(memory_space=pltpu.VMEM),
        out_shape=jax.ShapeDtypeStruct((1, 2 * M), _BF),
        scratch_shapes=[
            vmem((1, M), _BF), vmem((1, M), _BF),
            vmem((4, 8, W, D), _BF), vmem((4, 8, W, D), _BF),
            vmem((4, 128, H * D), _BF), vmem((32, 128, M), _BF), vmem((16, 256, C), _BF),
            vmem((4, 128, H, D), _BF), vmem((4, 128, H, D), _BF), vmem((4, 128, H, D), _BF),
            vmem((4, 1024, M), _BF),
            vmem((128, 128), _F32), vmem((H, C), _BF), vmem((16, H, 256), _F32), vmem((H, C), _F32),
            vmem((H, D), _F32), vmem((8, H, 128), _F32), vmem((H, D), _F32), vmem((H, D), _F32),
            vmem((8, 128), _F32), vmem((_NVPU, 128, 128), _F32),
            pltpu.SemaphoreType.DMA((2 * _NSEM,)), pltpu.SemaphoreType.DMA((2,)),
        ],
        compiler_params=pltpu.CompilerParams(
            vmem_limit_bytes=64 * 1024 * 1024,
            disable_bounds_checks=True,
            disable_semaphore_checks=True,
        ),
    )(
        A_x.reshape(1, M), A_k_cache, A_v_cache, A_wq.reshape(4, 128, H * D), A_wo.reshape(8, 512, M),
        B_x.reshape(1, M), B_c_kv.reshape(4, 1024, C),
        B_w_q.reshape(4, 128, H, D), B_w_uk.reshape(4, 128, H, D), B_w_uv.reshape(4, 128, H, D),
        B_w_o.reshape(4, 1024, M),
    )
    return out.reshape(1, 1, 2 * M)
```
